```python
import jax
import jax.numpy as jnp

def _softmax(x, axis=-1):
    return jax.nn.softmax(x, axis=axis)
def _gelu(x):
    return jax.nn.gelu(x, approximate=True)
def _silu(x):
    return jax.nn.silu(x)
def _sigmoid(x):
    return jax.nn.sigmoid(x)
def _layernorm(x, axis=-1, eps=1e-5):
    m = jnp.mean(x, axis=axis, keepdims=True)
    v = jnp.var(x, axis=axis, keepdims=True)
    return (x - m) / jnp.sqrt(v + eps)
def _scatter_add(tgt, idx, src, axis=0):
    return tgt.at[idx].add(src)
def _segment_sum(src, seg, n):
    return jax.ops.segment_sum(src, seg, n)
class _Rng:
    def __init__(self, key):
        self._k = key
    def _next(self):
        self._k, sub = jax.random.split(self._k)
        return sub
    def normal(self, shape):
        return jax.random.normal(self._next(), shape, dtype=jnp.bfloat16)
    def randint(self, lo, hi, shape):
        return jax.random.randint(self._next(), shape, lo, hi, dtype=jnp.int32)
    def uniform(self, shape, lo=0.0, hi=1.0):
        return jax.random.uniform(self._next(), shape, jnp.bfloat16, lo, hi)
    def permutation(self, n):
        return jax.random.permutation(self._next(), n)


kernel_name = 'sequential_preLN__sliding_block_cached__glu_gated_swiglu__decode'

def setup_inputs():
    _rng = _Rng(jax.random.key(int.from_bytes(__import__("os").urandom(4), "little")))
    _w = (lambda a: (lambda t: t.astype(jnp.bfloat16) if jnp.issubdtype(t.dtype, jnp.floating) else t)(jnp.asarray(a)))
    def _A_setup():
        B, Sq, D = 1, 1, 640
        Hq, Hkv, Sk, Dh = 32, 32, 32768, 192
        assert Hq % Hkv == 0, (Hq, Hkv)
        return {
            "x": _w((lambda *s: _rng.normal(s) * 0.05)(B, Sq, D)),
            "k_cache": _w((lambda *s: _rng.normal(s) * 0.05)(B, Hkv, Sk, Dh)),
            "v_cache": _w((lambda *s: _rng.normal(s) * 0.05)(B, Hkv, Sk, Dh)),
            "wq": _w((lambda *s: _rng.normal(s) * 0.05)(D, Hq * Dh) * (D ** -0.5)),
            "wo": _w((lambda *s: _rng.normal(s) * 0.05)(Hq * Dh, D) * ((Hq * Dh) ** -0.5)),
        }
    _A_in = _A_setup()

    def _B_setup():
        B, S, D, F = 1, 1, 640, 1536
        return {
            "x": _w((lambda *s: _rng.normal(s) * 0.05)(B, S, D)),
            "w1": _w((lambda *s: _rng.normal(s) * 0.05)(D, F) * (2.0 / D) ** 0.5),
            "w3": _w((lambda *s: _rng.normal(s) * 0.05)(D, F) * (2.0 / D) ** 0.5),
            "w2": _w((lambda *s: _rng.normal(s) * 0.05)(F, D) * (2.0 / F) ** 0.5),
        }
    _B_in = _B_setup()

    return {
        "A_x": _A_in["x"],
        "A_k_cache": _A_in["k_cache"],
        "A_v_cache": _A_in["v_cache"],
        "A_wq": _A_in["wq"],
        "A_wo": _A_in["wo"],
        "B_x": _B_in["x"],
        "B_w1": _B_in["w1"],
        "B_w3": _B_in["w3"],
        "B_w2": _B_in["w2"],
    }

def reference(A_x, A_k_cache, A_v_cache, A_wq, A_wo, B_x, B_w1, B_w3, B_w2):
    def _A_ref(x, k_cache, v_cache, wq, wo):
        B, Sq, D = x.shape
        Hq, Dh = 32, 192
        Hkv, Sk = k_cache.shape[1], k_cache.shape[2]
        W = min(4096, max(256, Sk // 4))
        rep = Hq // Hkv
        q = (lambda x, *d: x.transpose(*d))((x @ wq).reshape(B, Sq, Hq, Dh), 0, 2, 1, 3)
        k = jnp.repeat(k_cache[:, :, Sk - W:, :], rep, axis=1)
        v = jnp.repeat(v_cache[:, :, Sk - W:, :], rep, axis=1)
        scores = jnp.einsum("bhqd,bhkd->bhqk", q, k) * (Dh ** -0.5)
        p = _softmax(scores, axis=-1)
        o = jnp.einsum("bhqk,bhkd->bhqd", p, v)
        return (lambda x, *d: x.transpose(*d))(o, 0, 2, 1, 3).reshape(B, Sq, Hq * Dh) @ wo

    def _B_ref(x, w1, w3, w2):
        gate = jnp.einsum("bsd,df->bsf", x, w1)
        up = jnp.einsum("bsd,df->bsf", x, w3)
        h = _silu(gate) * up
        out = jnp.einsum("bsf,fd->bsd", h, w2)
        return out

    x = A_x
    h = x + _A_ref(_layernorm(x, axis=-1), A_k_cache, A_v_cache, A_wq, A_wo)
    h2 = h + _B_ref(_layernorm(h, axis=-1), B_w1, B_w3, B_w2)
    return h2
```

```python
import jax
import jax.numpy as jnp
import numpy as np
from jax import lax
import jax.experimental.pallas as pl
import jax.experimental.pallas.tpu as pltpu

H, DH, SK, D, F = 32, 192, 32768, 640, 1536
W = min(4096, max(256, SK // 4))
BF = jnp.bfloat16
F32 = jnp.float32

CH = 16
CW = CH * 128
HG = 4
NG = H // HG
G = HG * DH // 8
KS = G // 3
ROUNDS = (W // CW) * KS
DT, FT = D // 128, F // 128


def _bf16_round(v):
    u = int(np.float32(v).view(np.uint32))
    u = (u + 0x7FFF + ((u >> 16) & 1)) & 0xFFFF0000
    return float(np.uint32(u).view(np.float32))


SCALE = _bf16_round(DH ** -0.5)
EPS = _bf16_round(1e-5)


def _r(x):
    return x.astype(BF).astype(F32)


def _layernorm(x32):
    m = jnp.mean(x32, axis=-1, keepdims=True)
    c = x32 - m
    v = jnp.mean(c * c, axis=-1, keepdims=True)
    num = _r(x32 - _r(m))
    den = _r(jnp.sqrt(_r(_r(v) + EPS)))
    return (num / den).astype(BF)


def _tiles(a):
    r, c = a.shape
    return a.reshape(r // 8, 8, c // 128, 128).transpose(0, 2, 1, 3).reshape(r // 8 * (c // 128), 8, 128)


def _tile_dot(lhs, tiles, ncol):
    nrb = tiles.shape[0] // ncol
    t = tiles.reshape(nrb, ncol, 8, 128)
    return jnp.concatenate(
        [jnp.dot(lhs, t[:, j].reshape(nrb * 8, 128), preferred_element_type=F32) for j in range(ncol)], axis=1)


def _order(n, streams):
    step = -(-n // streams)
    return [b + step * i for b in range(step) for i in range(streams) if b + step * i < n]


def _cut(t0, n, parts):
    out = []
    while n:
        for p in (parts if n >= sum(parts) else (n,)):
            out.append((t0, p))
            t0, n = t0 + p, n - p
    return out


def _merge(a, b):
    out, ia, ib = [], 0, 0
    while ia < len(a) or ib < len(b):
        if ib >= len(b) or (ia < len(a) and ia * len(b) <= ib * len(a)):
            out += a[ia]
            ia += 1
        else:
            out += b[ib]
            ib += 1
    return out


def make_kernel(q_pat=(4, 3, (5, 11)), kv_pat=(52, (5, 11)), o_pat=(5, 3, (5, 11)), f_pat=(2, 5, (3, 13)),
                w2_mxu=(32, 32, 11), w2_vpu=(9, 6, 3, 3), mxu_parts=((16,), (6, 10)), vpu_parts=((15,), (2, 3)),
                kv_split=12, o_first=5, o_next=2, f_first=66, o_steps=4):
    RPH = ROUNDS // HG
    QR = D // 8 // 2
    OC = H * DH * D // 1024 // CH // 2
    FC = D * F // 1024 // CH // 2

    f_jobs = _merge([[(c * CH, CH, 0)] for c in _order(FC, f_pat[0])],
                    [[(t, n, 1) for t, n in _cut((FC + (c + f_pat[1]) % FC) * CH, CH, f_pat[2])]
                     for c in _order(FC, f_pat[0])])
    assert sum(w2_mxu + w2_vpu) == F // 8 // 2
    w2_groups, w2_jobs, rb = [], [], 0
    for i, n in enumerate(w2_mxu + w2_vpu):
        parts = mxu_parts if i < len(w2_mxu) else vpu_parts
        w2_groups.append(((rb, n), (F // 8 // 2 + rb, n)))
        w2_jobs.append(_merge(*[[[(t, m, thread)] for t, m in _cut(r0 * DT, n * DT, parts[thread])]
                                for thread, (r0, _) in enumerate(w2_groups[-1])]))
        rb += n

    def kernel(x_hbm, kt_hbm, vt_hbm, wq_hbm, wo_hbm, w1_hbm, w3_hbm, w2_hbm, o_hbm,
               x_v, wq_v, q_v, kbuf, vbuf, wo_v, w1_v, w3_v, w2_v, o_v, sem_o):

        def body(sem_x, sem_wq, sem_wo, sem_k, sem_v, sem_w1, sem_w3, sem_w2):
            def wait_all(ref, sem):
                pltpu.make_async_copy(ref, ref, sem).wait()

            def loop(lo, hi, fn):
                lax.fori_loop(lo, hi, lambda i, c: (fn(i), c)[1], 0)

            def wrap(i, n):
                return jnp.where(i >= n, i - n, i)

            def rows(rb):
                return pl.ds(pl.multiple_of(rb * 8, 8), 8)

            def cols(c, n):
                return pl.ds(pl.multiple_of(c, 128), n * 128)

            def tile_copy(src, dst, sem, t0, n, thread):
                sl = pl.ds(t0, n)
                pltpu.make_async_copy(src.at[sl], dst.at[sl], sem).start(priority=thread)

            def issue(*runs):
                runs = [run for run in runs if run[3]]

                def step(i):
                    for n, (src, dst, sem, jobs) in enumerate(runs):
                        @pl.when(i == n)
                        def _():
                            for job in jobs:
                                tile_copy(src, dst, sem, *job)

                if runs:
                    loop(0, max(len(runs), 2), step)

            def q_round(b):
                streams, off, parts = q_pat
                rb, c = b // 3, b % 3
                for i in range(streams):
                    r = rb + QR // streams * i
                    for thread, rr, pp in ((0, r, (CH,)), (1, QR + wrap(r + off, QR), parts)):
                        col = c * CW
                        for p in pp:
                            idx = (rows(rr), cols(col, p))
                            pltpu.make_async_copy(wq_hbm.at[idx], wq_v.at[idx], sem_wq).start(priority=thread)
                            col = col + p * 128

            def kv_round(g, t):
                off, parts = kv_pat
                slot, col0, b = g & 1, (t >> (KS.bit_length() - 1)) * CW, t & (KS - 1)
                for i in range(G // KS):
                    for thread, rb, pp, src, dst, sem in (
                            (0, b + KS * i, (CH,), vt_hbm, vbuf, sem_v),
                            (1, wrap(b + KS * i + off, G), parts, kt_hbm, kbuf, sem_k)):
                        col = col0
                        for p in pp:
                            pltpu.make_async_copy(src.at[rows(g * G + rb), cols(SK - W + col, p)],
                                                  dst.at[slot, rows(rb), cols(col, p)],
                                                  sem.at[slot]).start(priority=thread)
                            col = col + p * 128

            def o_round(b):
                streams, off, parts = o_pat
                for i in range(streams):
                    c = b + OC // streams * i
                    tile_copy(wo_hbm, wo_v, sem_wo, c * CH, CH, 0)
                    t0 = (OC + wrap(c + off, OC)) * CH
                    for p in parts:
                        tile_copy(wo_hbm, wo_v, sem_wo, t0, p, 1)
                        t0 = t0 + p

            x_copy = pltpu.make_async_copy(x_hbm, x_v, sem_x)
            x_copy.start()
            loop(0, 3 * QR // q_pat[0], q_round)
            x_copy.wait()
            x32 = x_v[...].astype(F32)
            lnx = jnp.broadcast_to(_layernorm(x32), (8, D))

            def q_part(j):
                loop(j * RPH, j * RPH + kv_split, lambda t: kv_round(0, t))

                @pl.when(j == 0)
                def _():
                    wait_all(wq_v, sem_wq)

                qc = jnp.dot(lnx, wq_v[:, pl.ds(pl.multiple_of(j * NG * DH, 128), NG * DH)],
                             preferred_element_type=F32)
                for i in range(NG):
                    q_v[j * NG + i] = qc[:, i * DH:(i + 1) * DH]
                loop(j * RPH + kv_split, (j + 1) * RPH, lambda t: kv_round(0, t))

            loop(0, HG, q_part)

            def head(h):
                g, j = h >> (HG.bit_length() - 1), h & (HG - 1)
                slot = g & 1
                more = g + 1 < NG

                def prefetch(lo, hi, o_lo, o_hi):
                    @pl.when(more)
                    def _():
                        loop(j * RPH + lo, j * RPH + hi, lambda t: kv_round(g + 1, t))

                    @pl.when(jnp.logical_not(more))
                    def _():
                        loop(o_lo, o_hi, o_round)

                o_mid = o_first + 2 * j * o_next
                prefetch(0, kv_split, jnp.where(j == 0, 0, o_mid - o_next), o_mid)

                @pl.when(j == 0)
                def _():
                    wait_all(vbuf.at[slot], sem_v.at[slot])
                    wait_all(kbuf.at[slot], sem_k.at[slot])

                hrows = pl.ds(pl.multiple_of(j * DH, DH), DH)
                qh = q_v[h].astype(BF)
                s = jnp.dot(qh, kbuf[slot, hrows, :], preferred_element_type=F32)
                s = _r(_r(s) * SCALE)
                m = jnp.max(s, axis=-1, keepdims=True)
                e = _r(jnp.exp(_r(s - m)))
                l = _r(jnp.sum(e, axis=-1, keepdims=True))
                p = (e / l).astype(BF)
                prefetch(kv_split, RPH, o_mid, o_mid + o_next)
                q_v[h] = lax.dot_general(p, vbuf[slot, hrows, :], (((1,), (1,)), ((), ())),
                                         preferred_element_type=F32)

            loop(0, H, head)
            loop(o_first + (2 * HG - 1) * o_next, OC // o_pat[0], o_round)

            def issue_f(lo, hi):
                n = len(f_jobs)
                issue((w1_hbm, w1_v, sem_w1, f_jobs[min(lo, n):min(hi, n)]),
                      (w3_hbm, w3_v, sem_w3, f_jobs[max(lo - n, 0):max(hi - n, 0)]))

            issue_f(0, f_first)
            wait_all(wo_v, sem_wo)
            hs = H // o_steps
            nf = -(-(2 * len(f_jobs) - f_first) // o_steps)
            attn = jnp.zeros((8, D), F32)
            for c in range(o_steps):
                o = jnp.concatenate([q_v[c * hs + i] for i in range(hs)], axis=1).astype(BF)
                nt = hs * DH // 8 * DT
                attn = attn + _tile_dot(o, wo_v[c * nt:(c + 1) * nt], DT)
                issue_f(f_first + c * nf, f_first + (c + 1) * nf)
            hres = _r(x32 + _r(attn))
            lnh = _layernorm(hres)

            wait_all(w1_v, sem_w1)
            gate = _r(_tile_dot(lnh, w1_v[...], FT))
            gate = _r(gate * _r(jax.nn.sigmoid(gate)))
            issue(*[(w2_hbm, w2_v, sem_w2.at[i], jobs) for i, jobs in enumerate(w2_jobs)])
            wait_all(w3_v, sem_w3)
            up = _r(_tile_dot(lnh, w3_v[...], FT))
            hm = (gate * up).astype(BF)
            h32 = hm[0:1].astype(F32)
            hcol = {}
            for group in w2_groups[len(w2_mxu):]:
                for r0, n in group:
                    for b in range(r0 // 16, (r0 + n - 1) // 16 + 1):
                        if b not in hcol:
                            hcol[b] = jnp.broadcast_to(h32[:, b * 128:(b + 1) * 128], (128, 128)).T
            out = jnp.zeros((8, D), F32)
            acc = [None] * DT
            for i, group in enumerate(w2_groups):
                for r0, n in group:
                    wait_all(w2_v.at[pl.ds(r0 * DT, n * DT)], sem_w2.at[i])
                for r0, n in group:
                    if i < len(w2_mxu):
                        out = out + _tile_dot(hm[:, r0 * 8:(r0 + n) * 8], w2_v[r0 * DT:(r0 + n) * DT], DT)
                    else:
                        for r in range(r0, r0 + n):
                            hb = hcol[r // 16][r % 16 * 8:(r % 16 + 1) * 8]
                            for c in range(DT):
                                term = hb * w2_v[r * DT + c].astype(F32)
                                acc[c] = term if acc[c] is None else acc[c] + term
            out = out[0:1] + jnp.concatenate([jnp.sum(a, axis=0, keepdims=True) for a in acc], axis=1)
            o_v[...] = (hres[0:1] + _r(out)).astype(o_v.dtype)
            pltpu.make_async_copy(o_v, o_hbm, sem_o).start()

        dma = pltpu.SemaphoreType.DMA
        pl.run_scoped(body, dma(()), dma(()), dma(()), dma((2,)), dma((2,)), dma(()), dma(()),
                      dma((len(w2_groups),)))
        pltpu.make_async_copy(o_v, o_hbm, sem_o).wait()

    @jax.jit
    def run(A_x, A_k_cache, A_v_cache, A_wq, A_wo, B_x, B_w1, B_w3, B_w2):
        del B_x
        x = A_x.reshape(1, D)
        kt = jnp.swapaxes(A_k_cache.reshape(H, SK, DH), 1, 2).reshape(H * DH, SK)
        vt = jnp.swapaxes(A_v_cache.reshape(H, SK, DH), 1, 2).reshape(H * DH, SK)
        tile_buf = lambda a: pltpu.VMEM((a.size // 1024, 8, 128), BF)
        out = pl.pallas_call(
            kernel,
            out_shape=jax.ShapeDtypeStruct((1, D), A_x.dtype),
            in_specs=[pl.BlockSpec(memory_space=pl.ANY)] * 8,
            out_specs=pl.BlockSpec(memory_space=pl.ANY),
            scratch_shapes=[
                pltpu.VMEM((1, D), BF),
                pltpu.VMEM((D, H * DH), BF),
                pltpu.VMEM((H, 8, DH), F32),
                pltpu.VMEM((2, HG * DH, W), BF),
                pltpu.VMEM((2, HG * DH, W), BF),
                tile_buf(A_wo), tile_buf(B_w1), tile_buf(B_w3), tile_buf(B_w2),
                pltpu.VMEM((1, D), BF),
                pltpu.SemaphoreType.DMA(()),
            ],
            compiler_params=pltpu.CompilerParams(vmem_limit_bytes=100 * 1024 * 1024, disable_bounds_checks=True),
        )(x, kt, vt, A_wq, _tiles(A_wo), _tiles(B_w1), _tiles(B_w3), _tiles(B_w2))
        return out.reshape(1, 1, D)

    return run


pallas_sequential_preLN__sliding_block_cached__glu_gated_swiglu__decode_kernel = make_kernel()
```

```python
import jax
import jax.numpy as jnp
import numpy as np
from jax import lax
import jax.experimental.pallas as pl
import jax.experimental.pallas.tpu as pltpu

H, DH, SK, D, F = 32, 192, 32768, 640, 1536
W = min(4096, max(256, SK // 4))
BF = jnp.bfloat16
F32 = jnp.float32

CH = 16
CW = CH * 128
HG = 4
NG = H // HG
G = HG * DH // 8
KS = G // 3
ROUNDS = (W // CW) * KS
DT, FT = D // 128, F // 128


def _bf16_round(v):
    u = int(np.float32(v).view(np.uint32))
    u = (u + 0x7FFF + ((u >> 16) & 1)) & 0xFFFF0000
    return float(np.uint32(u).view(np.float32))


SCALE = _bf16_round(DH ** -0.5)
EPS = _bf16_round(1e-5)


def _r(x):
    return x.astype(BF).astype(F32)


def _layernorm(x32):
    m = jnp.mean(x32, axis=-1, keepdims=True)
    c = x32 - m
    v = jnp.mean(c * c, axis=-1, keepdims=True)
    num = _r(x32 - _r(m))
    den = _r(jnp.sqrt(_r(_r(v) + EPS)))
    return (num / den).astype(BF)


def _tiles(a):
    r, c = a.shape
    return a.reshape(r // 8, 8, c // 128, 128).transpose(0, 2, 1, 3).reshape(r // 8 * (c // 128), 8, 128)


def _tile_dot(lhs, tiles, ncol):
    nrb = tiles.shape[0] // ncol
    t = tiles.reshape(nrb, ncol, 8, 128)
    return jnp.concatenate(
        [jnp.dot(lhs, t[:, j].reshape(nrb * 8, 128), preferred_element_type=F32) for j in range(ncol)], axis=1)


def _order(n, streams):
    step = -(-n // streams)
    return [b + step * i for b in range(step) for i in range(streams) if b + step * i < n]


def _cut(t0, n, parts, phase):
    out, end = [], t0 + n
    while t0 < end:
        m = min(end - t0, CH - (t0 - phase) % CH)
        for p in (parts if m == CH else (m,)):
            out.append((t0, p))
            t0 += p
    return out


def _merge(a, b):
    out, ia, ib = [], 0, 0
    while ia < len(a) or ib < len(b):
        if ib >= len(b) or (ia < len(a) and ia * len(b) <= ib * len(a)):
            out += a[ia]
            ia += 1
        else:
            out += b[ib]
            ib += 1
    return out


def _weight_jobs(chunks, streams, off, parts, phase):
    half = chunks // 2

    def second(c):
        if c < chunks - 1 or not phase:
            return _cut(phase + c * CH, CH, parts, phase)
        return [(phase + c * CH, CH - phase), (0, phase)]

    order = _order(half, streams)
    return _merge([[(phase + c * CH, CH, 0)] for c in order],
                  [[(t, n, 1) for t, n in second(half + (c + off) % half)] for c in order])


def make_kernel(q_pat=(4, 3, (5, 11), 0), o_pat=(5, 3, (5, 11), 0), w1_pat=(2, 5, (3, 13), 0),
                w3_pat=(2, 5, (3, 13), 0), w2_pat=((6, 10), 0), kv_pat=(52, 1, (8, 3, 5)),
                w2_mxu=(32, 32, 11), w2_vpu=(9, 6, 3, 3),
                kv_split=12, o_first=75, o_next=30, f_first=66, o_steps=4):
    RPH = ROUNDS // HG
    q_jobs = _weight_jobs(D * H * DH // 1024 // CH, *q_pat)
    o_jobs = _weight_jobs(D * H * DH // 1024 // CH, *o_pat)
    w1_jobs = _weight_jobs(D * F // 1024 // CH, *w1_pat)
    w3_jobs = _weight_jobs(D * F // 1024 // CH, *w3_pat)
    assert sum(w2_mxu + w2_vpu) == F // 8 // 2
    w2_groups, w2_jobs, rb = [], [], 0
    for i, n in enumerate(w2_mxu + w2_vpu):
        r1 = F // 8 // 2 + rb
        w2_groups.append(((rb, n), (r1, n)))
        if i < len(w2_mxu):
            first = _cut(rb * DT, n * DT, (CH,), w2_pat[1])
            second = _cut(r1 * DT, n * DT, w2_pat[0], w2_pat[1])
        else:
            first = [(r * DT, 3 * DT) for r in range(rb, rb + n, 3)]
            second = [p for r in range(r1, r1 + n) for p in ((r * DT, 2), (r * DT + 2, DT - 2))]
        w2_jobs.append(_merge([[(t, m, 0)] for t, m in first], [[(t, m, 1)] for t, m in second]))
        rb += n

    def kernel(x_hbm, kt_hbm, vt_hbm, wq_hbm, wo_hbm, w1_hbm, w3_hbm, w2_hbm, o_hbm,
               x_v, wq_v, q_v, kbuf, vbuf, wo_v, w1_v, w3_v, w2_v, o_v, sem_o):

        def body(sem_x, sem_wq, sem_wo, sem_k, sem_v, sem_w1, sem_w3, sem_w2):
            def wait_all(ref, sem):
                pltpu.make_async_copy(ref, ref, sem).wait()

            def loop(lo, hi, fn):
                lax.fori_loop(lo, hi, lambda i, c: (fn(i), c)[1], 0)

            def wrap(i, n):
                return jnp.where(i >= n, i - n, i)

            def rows(rb):
                return pl.ds(pl.multiple_of(rb * 8, 8), 8)

            def tile_copy(src, dst, sem, t0, n, thread):
                sl = pl.ds(t0, n)
                pltpu.make_async_copy(src.at[sl], dst.at[sl], sem).start(priority=thread)

            def issue(*runs):
                runs = [run for run in runs if run[3]]

                def step(i):
                    for n, (src, dst, sem, jobs) in enumerate(runs):
                        @pl.when(i == n)
                        def _():
                            for job in jobs:
                                tile_copy(src, dst, sem, *job)

                if runs:
                    loop(0, max(len(runs), 2), step)

            def kv_round(g, t):
                off, flip, parts = kv_pat
                slot, half, b = g & 1, t >> (KS.bit_length() - 1), t & (KS - 1)
                for i in range(3):
                    k = 2 * (3 * b + i)
                    rb = jnp.where(k >= G, k - (G - 1), k)
                    for thread, r, c, pieces, src, dst, sem in (
                            (0, rb, half, (CH,), kt_hbm, kbuf, sem_k),
                            (1, wrap(rb + off, G), half ^ flip, parts, vt_hbm, vbuf, sem_v)):
                        col = c * CW
                        for n in pieces:
                            pltpu.make_async_copy(
                                src.at[rows(g * G + r), pl.ds(pl.multiple_of(SK - W + col, 128), n * 128)],
                                dst.at[slot, rows(r), pl.ds(pl.multiple_of(col, 128), n * 128)],
                                sem.at[slot]).start(priority=thread)
                            col = col + n * 128

            x_copy = pltpu.make_async_copy(x_hbm, x_v, sem_x)
            x_copy.start()
            issue((wq_hbm, wq_v, sem_wq, q_jobs))
            x_copy.wait()
            x32 = x_v[...].astype(F32)
            lnx = jnp.broadcast_to(_layernorm(x32), (8, D))

            for j in range(HG):
                loop(j * RPH, j * RPH + kv_split, lambda t: kv_round(0, t))
                if j == 0:
                    wait_all(wq_v, sem_wq)
                nc = NG * DH // 128
                t = wq_v[...].reshape(D // 8, HG * nc, 8, 128)
                qc = jnp.concatenate([jnp.dot(lnx, t[:, c].reshape(D, 128), preferred_element_type=F32)
                                      for c in range(j * nc, (j + 1) * nc)], axis=1)
                for i in range(NG):
                    q_v[j * NG + i] = qc[:, i * DH:(i + 1) * DH]
                loop(j * RPH + kv_split, (j + 1) * RPH, lambda t: kv_round(0, t))

            def head(h):
                g, j = h >> (HG.bit_length() - 1), h & (HG - 1)
                slot = g & 1
                more = g + 1 < NG

                def prefetch(lo, hi, part):
                    @pl.when(more)
                    def _():
                        loop(j * RPH + lo, j * RPH + hi, lambda t: kv_round(g + 1, t))

                    for i in range(HG):
                        @pl.when(h == H - HG + i)
                        def _():
                            end = o_first + (2 * i + part) * o_next
                            for job in o_jobs[end - o_next if 2 * i + part else 0:end]:
                                tile_copy(wo_hbm, wo_v, sem_wo, *job)

                prefetch(0, kv_split, 0)

                @pl.when(j == 0)
                def _():
                    wait_all(vbuf.at[slot], sem_v.at[slot])
                    wait_all(kbuf.at[slot], sem_k.at[slot])

                hrows = pl.ds(pl.multiple_of(j * DH, DH), DH)
                qh = q_v[h].astype(BF)
                s = jnp.dot(qh, kbuf[slot, hrows, :], preferred_element_type=F32)
                s = _r(_r(s) * SCALE)
                m = jnp.max(s, axis=-1, keepdims=True)
                e = _r(jnp.exp(_r(s - m)))
                l = _r(jnp.sum(e, axis=-1, keepdims=True))
                p = (e / l).astype(BF)
                prefetch(kv_split, RPH, 1)
                q_v[h] = lax.dot_general(p, vbuf[slot, hrows, :], (((1,), (1,)), ((), ())),
                                         preferred_element_type=F32)

            loop(0, H, head)
            issue((wo_hbm, wo_v, sem_wo, o_jobs[o_first + (2 * HG - 1) * o_next:]))

            def issue_f(lo, hi):
                n = len(w1_jobs)
                issue((w1_hbm, w1_v, sem_w1, w1_jobs[min(lo, n):min(hi, n)]),
                      (w3_hbm, w3_v, sem_w3, w3_jobs[max(lo - n, 0):max(hi - n, 0)]))

            issue_f(0, f_first)
            wait_all(wo_v, sem_wo)
            hs = H // o_steps
            nf = -(-(len(w1_jobs) + len(w3_jobs) - f_first) // o_steps)
            attn = jnp.zeros((8, D), F32)
            for c in range(o_steps):
                o = jnp.concatenate([q_v[c * hs + i] for i in range(hs)], axis=1).astype(BF)
                nt = hs * DH // 8 * DT
                attn = attn + _tile_dot(o, wo_v[c * nt:(c + 1) * nt], DT)
                issue_f(f_first + c * nf, f_first + (c + 1) * nf)
            hres = _r(x32 + _r(attn))
            lnh = _layernorm(hres)

            wait_all(w1_v, sem_w1)
            gate = _r(_tile_dot(lnh, w1_v[...], FT))
            gate = _r(gate * _r(jax.nn.sigmoid(gate)))
            issue(*[(w2_hbm, w2_v, sem_w2.at[i], jobs) for i, jobs in enumerate(w2_jobs)])
            wait_all(w3_v, sem_w3)
            up = _r(_tile_dot(lnh, w3_v[...], FT))
            hm = (gate * up).astype(BF)
            h32 = hm[0:1].astype(F32)
            hcol = {}
            for group in w2_groups[len(w2_mxu):]:
                for r0, n in group:
                    for b in range(r0 // 16, (r0 + n - 1) // 16 + 1):
                        if b not in hcol:
                            hcol[b] = jnp.broadcast_to(h32[:, b * 128:(b + 1) * 128], (128, 128)).T
            out = jnp.zeros((8, D), F32)
            acc = [None] * DT
            for i, group in enumerate(w2_groups):
                for r0, n in group:
                    wait_all(w2_v.at[pl.ds(r0 * DT, n * DT)], sem_w2.at[i])
                for r0, n in group:
                    if i < len(w2_mxu):
                        out = out + _tile_dot(hm[:, r0 * 8:(r0 + n) * 8], w2_v[r0 * DT:(r0 + n) * DT], DT)
                    else:
                        for r in range(r0, r0 + n):
                            hb = hcol[r // 16][r % 16 * 8:(r % 16 + 1) * 8]
                            for c in range(DT):
                                term = hb * w2_v[r * DT + c].astype(F32)
                                acc[c] = term if acc[c] is None else acc[c] + term
            out = out[0:1] + jnp.concatenate([jnp.sum(a, axis=0, keepdims=True) for a in acc], axis=1)
            o_v[...] = (hres[0:1] + _r(out)).astype(o_v.dtype)
            pltpu.make_async_copy(o_v, o_hbm, sem_o).start()

        dma = pltpu.SemaphoreType.DMA
        pl.run_scoped(body, dma(()), dma(()), dma(()), dma((2,)), dma((2,)), dma(()), dma(()),
                      dma((len(w2_groups),)))
        pltpu.make_async_copy(o_v, o_hbm, sem_o).wait()

    @jax.jit
    def run(A_x, A_k_cache, A_v_cache, A_wq, A_wo, B_x, B_w1, B_w3, B_w2):
        del B_x
        x = A_x.reshape(1, D)
        kt = jnp.swapaxes(A_k_cache.reshape(H, SK, DH), 1, 2).reshape(H * DH, SK)
        vt = jnp.swapaxes(A_v_cache.reshape(H, SK, DH), 1, 2).reshape(H * DH, SK)
        tile_buf = lambda a: pltpu.VMEM((a.size // 1024, 8, 128), BF)
        out = pl.pallas_call(
            kernel,
            out_shape=jax.ShapeDtypeStruct((1, D), A_x.dtype),
            in_specs=[pl.BlockSpec(memory_space=pl.ANY)] * 8,
            out_specs=pl.BlockSpec(memory_space=pl.ANY),
            scratch_shapes=[
                pltpu.VMEM((1, D), BF),
                tile_buf(A_wq),
                pltpu.VMEM((H, 8, DH), F32),
                pltpu.VMEM((2, HG * DH, W), BF),
                pltpu.VMEM((2, HG * DH, W), BF),
                tile_buf(A_wo), tile_buf(B_w1), tile_buf(B_w3), tile_buf(B_w2),
                pltpu.VMEM((1, D), BF),
                pltpu.SemaphoreType.DMA(()),
            ],
            compiler_params=pltpu.CompilerParams(vmem_limit_bytes=100 * 1024 * 1024, disable_bounds_checks=True),
        )(x, kt, vt, _tiles(A_wq), _tiles(A_wo), _tiles(B_w1), _tiles(B_w3), _tiles(B_w2))
        return out.reshape(1, 1, D)

    return run


pallas_sequential_preLN__sliding_block_cached__glu_gated_swiglu__decode_kernel = make_kernel()
```

```python
import jax
import jax.numpy as jnp
import numpy as np
from jax import lax
import jax.experimental.pallas as pl
import jax.experimental.pallas.tpu as pltpu

H, DH, SK, D, F = 32, 192, 32768, 640, 1536
W = min(4096, max(256, SK // 4))
BF = jnp.bfloat16
F32 = jnp.float32

CH = 16
CW = CH * 128
HG = 4
NG = H // HG
G = HG * DH // 8
KS = G // 3
ROUNDS = (W // CW) * KS
DT, FT = D // 128, F // 128


def _bf16_round(v):
    u = int(np.float32(v).view(np.uint32))
    u = (u + 0x7FFF + ((u >> 16) & 1)) & 0xFFFF0000
    return float(np.uint32(u).view(np.float32))


SCALE = _bf16_round(DH ** -0.5)
EPS = _bf16_round(1e-5)


def _r(x):
    return x.astype(BF).astype(F32)


def _layernorm(x32):
    m = jnp.mean(x32, axis=-1, keepdims=True)
    c = x32 - m
    v = jnp.mean(c * c, axis=-1, keepdims=True)
    num = _r(x32 - _r(m))
    den = _r(jnp.sqrt(_r(_r(v) + EPS)))
    return (num / den).astype(BF)


def _tiles(a):
    r, c = a.shape
    return a.reshape(r // 8, 8, c // 128, 128).transpose(0, 2, 1, 3).reshape(r // 8 * (c // 128), 8, 128)


def _tile_dot(lhs, tiles, ncol):
    nrb = tiles.shape[0] // ncol
    t = tiles.reshape(nrb, ncol, 8, 128)
    return jnp.concatenate(
        [jnp.dot(lhs, t[:, j].reshape(nrb * 8, 128), preferred_element_type=F32) for j in range(ncol)], axis=1)


def _order(n, streams):
    step = -(-n // streams)
    return [b + step * i for b in range(step) for i in range(streams) if b + step * i < n]


def _cut(t0, n, parts, phase):
    out, end = [], t0 + n
    while t0 < end:
        m = min(end - t0, CH - (t0 - phase) % CH)
        for p in (parts if m == CH else (m,)):
            out.append((t0, p))
            t0 += p
    return out


def _merge(a, b):
    out, ia, ib = [], 0, 0
    while ia < len(a) or ib < len(b):
        if ib >= len(b) or (ia < len(a) and ia * len(b) <= ib * len(a)):
            out += a[ia]
            ia += 1
        else:
            out += b[ib]
            ib += 1
    return out


def _weight_jobs(chunks, streams, off, parts, phase):
    half = chunks // 2

    def second(c):
        if c < chunks - 1 or not phase:
            return _cut(phase + c * CH, CH, parts, phase)
        return [(phase + c * CH, CH - phase), (0, phase)]

    order = _order(half, streams)
    return _merge([[(phase + c * CH, CH, 0)] for c in order],
                  [[(t, n, 1) for t, n in second(half + (c + off) % half)] for c in order])


def make_kernel(q_pat=(5, 2, (6, 10), 0), o_pat=(5, 13, (8, 8), 0), w1_pat=(2, 5, (3, 13), 0),
                w3_pat=(2, 5, (3, 13), 0), w2_pat=((8, 8), 8), kv_pat=(39, 1, (6, 10), 0),
                w2_mxu=(32, 32, 11), w2_vpu=(9, 6, 3, 3),
                kv_split=12, o_first=75, o_next=30, f_first=66, o_steps=4):
    RPH = ROUNDS // HG
    q_jobs = _weight_jobs(D * H * DH // 1024 // CH, *q_pat)
    o_jobs = _weight_jobs(D * H * DH // 1024 // CH, *o_pat)
    w1_jobs = _weight_jobs(D * F // 1024 // CH, *w1_pat)
    w3_jobs = _weight_jobs(D * F // 1024 // CH, *w3_pat)
    assert sum(w2_mxu + w2_vpu) == F // 8 // 2
    w2_groups, w2_jobs, rb = [], [], 0
    for i, n in enumerate(w2_mxu + w2_vpu):
        r1 = F // 8 // 2 + rb
        w2_groups.append(((rb, n), (r1, n)))
        if i < len(w2_mxu):
            first = _cut(rb * DT, n * DT, (CH,), w2_pat[1])
            second = _cut(r1 * DT, n * DT, w2_pat[0], w2_pat[1])
        else:
            first = [(r * DT, 3 * DT) for r in range(rb, rb + n, 3)]
            second = [p for r in range(r1, r1 + n) for p in ((r * DT, 2), (r * DT + 2, DT - 2))]
        w2_jobs.append(_merge([[(t, m, 0)] for t, m in first], [[(t, m, 1)] for t, m in second]))
        rb += n

    def kernel(x_hbm, kt_hbm, vt_hbm, wq_hbm, wo_hbm, w1_hbm, w3_hbm, w2_hbm, o_hbm,
               x_v, wq_v, q_v, kbuf, vbuf, wo_v, w1_v, w3_v, w2_v, o_v, sem_o):

        def body(sem_x, sem_wq, sem_wo, sem_k, sem_v, sem_w1, sem_w3, sem_w2):
            def wait_all(ref, sem):
                pltpu.make_async_copy(ref, ref, sem).wait()

            def loop(lo, hi, fn):
                lax.fori_loop(lo, hi, lambda i, c: (fn(i), c)[1], 0)

            def wrap(i, n):
                return jnp.where(i >= n, i - n, i)

            def rows(rb):
                return pl.ds(pl.multiple_of(rb * 8, 8), 8)

            def tile_copy(src, dst, sem, t0, n, thread):
                sl = pl.ds(t0, n)
                pltpu.make_async_copy(src.at[sl], dst.at[sl], sem).start(priority=thread)

            def issue(*runs):
                runs = [run for run in runs if run[3]]

                def step(i):
                    for n, (src, dst, sem, jobs) in enumerate(runs):
                        @pl.when(i == n)
                        def _():
                            for job in jobs:
                                tile_copy(src, dst, sem, *job)

                if runs:
                    loop(0, max(len(runs), 2), step)

            def kv_round(g, t):
                off, flip, parts, swap = kv_pat
                slot, half, b = g & 1, t >> (KS.bit_length() - 1), t & (KS - 1)
                for i in range(3):
                    k = 2 * (3 * b + i)
                    rb = jnp.where(k >= G, k - (G - 1), k)
                    for thread, r, c, pieces in ((0, rb, half, (CH,)), (1, wrap(rb + off, G), half ^ flip, parts)):
                        src, dst, sem = ((kt_hbm, kbuf, sem_k), (vt_hbm, vbuf, sem_v))[thread ^ swap]
                        col = c * CW
                        for n in pieces:
                            pltpu.make_async_copy(
                                src.at[rows(g * G + r), pl.ds(pl.multiple_of(SK - W + col, 128), n * 128)],
                                dst.at[slot, rows(r), pl.ds(pl.multiple_of(col, 128), n * 128)],
                                sem.at[slot]).start(priority=thread)
                            col = col + n * 128

            x_copy = pltpu.make_async_copy(x_hbm, x_v, sem_x)
            x_copy.start()
            issue((wq_hbm, wq_v, sem_wq, q_jobs))
            x_copy.wait()
            x32 = x_v[...].astype(F32)
            lnx = jnp.broadcast_to(_layernorm(x32), (8, D))

            for j in range(HG):
                loop(j * RPH, j * RPH + kv_split, lambda t: kv_round(0, t))
                if j == 0:
                    wait_all(wq_v, sem_wq)
                nc = NG * DH // 128
                t = wq_v[...].reshape(D // 8, HG * nc, 8, 128)
                qc = jnp.concatenate([jnp.dot(lnx, t[:, c].reshape(D, 128), preferred_element_type=F32)
                                      for c in range(j * nc, (j + 1) * nc)], axis=1)
                for i in range(NG):
                    q_v[j * NG + i] = qc[:, i * DH:(i + 1) * DH]
                loop(j * RPH + kv_split, (j + 1) * RPH, lambda t: kv_round(0, t))

            def head(h):
                g, j = h >> (HG.bit_length() - 1), h & (HG - 1)
                slot = g & 1
                more = g + 1 < NG

                def prefetch(lo, hi, part):
                    @pl.when(more)
                    def _():
                        loop(j * RPH + lo, j * RPH + hi, lambda t: kv_round(g + 1, t))

                    for i in range(HG):
                        @pl.when(h == H - HG + i)
                        def _():
                            end = o_first + (2 * i + part) * o_next
                            for job in o_jobs[end - o_next if 2 * i + part else 0:end]:
                                tile_copy(wo_hbm, wo_v, sem_wo, *job)

                prefetch(0, kv_split, 0)

                @pl.when(j == 0)
                def _():
                    wait_all(vbuf.at[slot], sem_v.at[slot])
                    wait_all(kbuf.at[slot], sem_k.at[slot])

                hrows = pl.ds(pl.multiple_of(j * DH, DH), DH)
                qh = q_v[h].astype(BF)
                s = jnp.dot(qh, kbuf[slot, hrows, :], preferred_element_type=F32)
                s = _r(_r(s) * SCALE)
                m = jnp.max(s, axis=-1, keepdims=True)
                e = _r(jnp.exp(_r(s - m)))
                l = _r(jnp.sum(e, axis=-1, keepdims=True))
                p = (e / l).astype(BF)
                prefetch(kv_split, RPH, 1)
                q_v[h] = lax.dot_general(p, vbuf[slot, hrows, :], (((1,), (1,)), ((), ())),
                                         preferred_element_type=F32)

            loop(0, H, head)
            issue((wo_hbm, wo_v, sem_wo, o_jobs[o_first + (2 * HG - 1) * o_next:]))

            def issue_f(lo, hi):
                n = len(w1_jobs)
                issue((w1_hbm, w1_v, sem_w1, w1_jobs[min(lo, n):min(hi, n)]),
                      (w3_hbm, w3_v, sem_w3, w3_jobs[max(lo - n, 0):max(hi - n, 0)]))

            issue_f(0, f_first)
            wait_all(wo_v, sem_wo)
            hs = H // o_steps
            nf = -(-(len(w1_jobs) + len(w3_jobs) - f_first) // o_steps)
            attn = jnp.zeros((8, D), F32)
            for c in range(o_steps):
                o = jnp.concatenate([q_v[c * hs + i] for i in range(hs)], axis=1).astype(BF)
                nt = hs * DH // 8 * DT
                attn = attn + _tile_dot(o, wo_v[c * nt:(c + 1) * nt], DT)
                issue_f(f_first + c * nf, f_first + (c + 1) * nf)
            hres = _r(x32 + _r(attn))
            lnh = _layernorm(hres)

            wait_all(w1_v, sem_w1)
            gate = _r(_tile_dot(lnh, w1_v[...], FT))
            gate = _r(gate * _r(jax.nn.sigmoid(gate)))
            issue(*[(w2_hbm, w2_v, sem_w2.at[i], jobs) for i, jobs in enumerate(w2_jobs)])
            wait_all(w3_v, sem_w3)
            up = _r(_tile_dot(lnh, w3_v[...], FT))
            hm = (gate * up).astype(BF)
            h32 = hm[0:1].astype(F32)
            hcol = {}
            for group in w2_groups[len(w2_mxu):]:
                for r0, n in group:
                    for b in range(r0 // 16, (r0 + n - 1) // 16 + 1):
                        if b not in hcol:
                            hcol[b] = jnp.broadcast_to(h32[:, b * 128:(b + 1) * 128], (128, 128)).T
            out = jnp.zeros((8, D), F32)
            acc = [None] * DT
            for i, group in enumerate(w2_groups):
                for r0, n in group:
                    wait_all(w2_v.at[pl.ds(r0 * DT, n * DT)], sem_w2.at[i])
                for r0, n in group:
                    if i < len(w2_mxu):
                        out = out + _tile_dot(hm[:, r0 * 8:(r0 + n) * 8], w2_v[r0 * DT:(r0 + n) * DT], DT)
                    else:
                        for r in range(r0, r0 + n):
                            hb = hcol[r // 16][r % 16 * 8:(r % 16 + 1) * 8]
                            for c in range(DT):
                                term = hb * w2_v[r * DT + c].astype(F32)
                                acc[c] = term if acc[c] is None else acc[c] + term
            out = out[0:1] + jnp.concatenate([jnp.sum(a, axis=0, keepdims=True) for a in acc], axis=1)
            o_v[...] = (hres[0:1] + _r(out)).astype(o_v.dtype)
            pltpu.make_async_copy(o_v, o_hbm, sem_o).start()

        dma = pltpu.SemaphoreType.DMA
        pl.run_scoped(body, dma(()), dma(()), dma(()), dma((2,)), dma((2,)), dma(()), dma(()),
                      dma((len(w2_groups),)))
        pltpu.make_async_copy(o_v, o_hbm, sem_o).wait()

    @jax.jit
    def run(A_x, A_k_cache, A_v_cache, A_wq, A_wo, B_x, B_w1, B_w3, B_w2):
        del B_x
        x = A_x.reshape(1, D)
        kt = jnp.swapaxes(A_k_cache.reshape(H, SK, DH), 1, 2).reshape(H * DH, SK)
        vt = jnp.swapaxes(A_v_cache.reshape(H, SK, DH), 1, 2).reshape(H * DH, SK)
        tile_buf = lambda a: pltpu.VMEM((a.size // 1024, 8, 128), BF)
        out = pl.pallas_call(
            kernel,
            out_shape=jax.ShapeDtypeStruct((1, D), A_x.dtype),
            in_specs=[pl.BlockSpec(memory_space=pl.ANY)] * 8,
            out_specs=pl.BlockSpec(memory_space=pl.ANY),
            scratch_shapes=[
                pltpu.VMEM((1, D), BF),
                tile_buf(A_wq),
                pltpu.VMEM((H, 8, DH), F32),
                pltpu.VMEM((2, HG * DH, W), BF),
                pltpu.VMEM((2, HG * DH, W), BF),
                tile_buf(A_wo), tile_buf(B_w1), tile_buf(B_w3), tile_buf(B_w2),
                pltpu.VMEM((1, D), BF),
                pltpu.SemaphoreType.DMA(()),
            ],
            compiler_params=pltpu.CompilerParams(vmem_limit_bytes=100 * 1024 * 1024, disable_bounds_checks=True),
        )(x, kt, vt, _tiles(A_wq), _tiles(A_wo), _tiles(B_w1), _tiles(B_w3), _tiles(B_w2))
        return out.reshape(1, 1, D)

    return run


pallas_sequential_preLN__sliding_block_cached__glu_gated_swiglu__decode_kernel = make_kernel()
```

```python
import jax
import jax.numpy as jnp
import numpy as np
from jax import lax
import jax.experimental.pallas as pl
import jax.experimental.pallas.tpu as pltpu

H, DH, SK, D, F = 32, 192, 32768, 640, 1536
W = min(4096, max(256, SK // 4))
BF = jnp.bfloat16
F32 = jnp.float32

CH = 16
CW = CH * 128
HG = 4
NG = H // HG
G = HG * DH // 8
KS = G // 3
ROUNDS = (W // CW) * KS
DT, FT = D // 128, F // 128


def _bf16_round(v):
    u = int(np.float32(v).view(np.uint32))
    u = (u + 0x7FFF + ((u >> 16) & 1)) & 0xFFFF0000
    return float(np.uint32(u).view(np.float32))


SCALE = _bf16_round(DH ** -0.5)
EPS = _bf16_round(1e-5)


def _r(x):
    return x.astype(BF).astype(F32)


def _layernorm(x32):
    m = jnp.mean(x32, axis=-1, keepdims=True)
    c = x32 - m
    v = jnp.mean(c * c, axis=-1, keepdims=True)
    num = _r(x32 - _r(m))
    den = _r(jnp.sqrt(_r(_r(v) + EPS)))
    return (num / den).astype(BF)


def _tiles(a):
    r, c = a.shape
    return a.reshape(r // 8, 8, c // 128, 128).transpose(0, 2, 1, 3).reshape(r // 8 * (c // 128), 8, 128)


def _tile_dot(lhs, tiles, ncol):
    nrb = tiles.shape[0] // ncol
    t = tiles.reshape(nrb, ncol, 8, 128)
    return jnp.concatenate(
        [jnp.dot(lhs, t[:, j].reshape(nrb * 8, 128), preferred_element_type=F32) for j in range(ncol)], axis=1)


def _order(n, streams):
    step = -(-n // streams)
    return [b + step * i for b in range(step) for i in range(streams) if b + step * i < n]


def _cut(t0, n, parts, phase):
    out, end = [], t0 + n
    while t0 < end:
        m = min(end - t0, CH - (t0 - phase) % CH)
        for p in (parts if m == CH else (m,)):
            out.append((t0, p))
            t0 += p
    return out


def _merge(a, b):
    out, ia, ib = [], 0, 0
    while ia < len(a) or ib < len(b):
        if ib >= len(b) or (ia < len(a) and ia * len(b) <= ib * len(a)):
            out += a[ia]
            ia += 1
        else:
            out += b[ib]
            ib += 1
    return out


def _weight_jobs(chunks, streams, off, parts, phase):
    half = chunks // 2

    def second(c):
        if c < chunks - 1 or not phase:
            return _cut(phase + c * CH, CH, parts, phase)
        return [(phase + c * CH, CH - phase), (0, phase)]

    order = _order(half, streams)
    return _merge([[(phase + c * CH, CH, 0)] for c in order],
                  [[(t, n, 1) for t, n in second(half + (c + off) % half)] for c in order])


def make_kernel(q_pat=(5, 2, (6, 10), 0), o_pat=(5, 13, (8, 8), 0), w1_pat=(2, 5, (3, 13), 0),
                w3_pat=(2, 5, (3, 13), 0), w2_pat=((10, 6), 0), kv_pat=(75, 0, (9, 7), 1),
                w2_mxu=(32, 32, 8), w2_vpu=(9, 6, 3, 3, 3),
                kv_split=12, o_first=75, o_next=33, f_first=80, o_steps=4):
    RPH = ROUNDS // HG
    q_jobs = _weight_jobs(D * H * DH // 1024 // CH, *q_pat)
    o_jobs = _weight_jobs(D * H * DH // 1024 // CH, *o_pat)
    w1_jobs = _weight_jobs(D * F // 1024 // CH, *w1_pat)
    w3_jobs = _weight_jobs(D * F // 1024 // CH, *w3_pat)
    assert sum(w2_mxu + w2_vpu) == F // 8 // 2 and all(n % 3 == 0 for n in w2_vpu)
    w2_groups, w2_jobs, rb = [], [], 0
    for i, n in enumerate(w2_mxu + w2_vpu):
        r1 = F // 8 // 2 + rb
        w2_groups.append(((rb, n), (r1, n)))
        if i < len(w2_mxu):
            first = _cut(rb * DT, n * DT, (CH,), w2_pat[1])
            second = _cut(r1 * DT, n * DT, w2_pat[0], w2_pat[1])
        else:
            first = [(r * DT, 3 * DT) for r in range(rb, rb + n, 3)]
            second = [p for r in range(r1, r1 + n) for p in ((r * DT, 2), (r * DT + 2, DT - 2))]
        w2_jobs.append(_merge([[(t, m, 0)] for t, m in first], [[(t, m, 1)] for t, m in second]))
        rb += n

    def kernel(x_hbm, kt_hbm, vt_hbm, wq_hbm, wo_hbm, w1_hbm, w3_hbm, w2_hbm, o_hbm,
               x_v, wq_v, q_v, kbuf, vbuf, wo_v, w1_v, w3_v, w2_v, o_v, sem_o):

        def body(sem_x, sem_wq, sem_wo, sem_k, sem_v, sem_w1, sem_w3, sem_w2):
            def wait_all(ref, sem):
                pltpu.make_async_copy(ref, ref, sem).wait()

            def loop(lo, hi, fn):
                lax.fori_loop(lo, hi, lambda i, c: (fn(i), c)[1], 0)

            def wrap(i, n):
                return jnp.where(i >= n, i - n, i)

            def rows(rb):
                return pl.ds(pl.multiple_of(rb * 8, 8), 8)

            def tile_copy(src, dst, sem, t0, n, thread):
                sl = pl.ds(t0, n)
                pltpu.make_async_copy(src.at[sl], dst.at[sl], sem).start(priority=thread)

            def issue(*runs):
                runs = [run for run in runs if run[3]]

                def step(i):
                    for n, (src, dst, sem, jobs) in enumerate(runs):
                        @pl.when(i == n)
                        def _():
                            for job in jobs:
                                tile_copy(src, dst, sem, *job)

                if runs:
                    loop(0, max(len(runs), 2), step)

            def kv_round(g, t):
                off, flip, parts, swap = kv_pat
                slot, half, b = g & 1, t >> (KS.bit_length() - 1), t & (KS - 1)
                for i in range(3):
                    k = 2 * (3 * b + i)
                    rb = jnp.where(k >= G, k - (G - 1), k)
                    for thread, r, c, pieces in ((0, rb, half, (CH,)), (1, wrap(rb + off, G), half ^ flip, parts)):
                        src, dst, sem = ((kt_hbm, kbuf, sem_k), (vt_hbm, vbuf, sem_v))[thread ^ swap]
                        col = c * CW
                        for n in pieces:
                            pltpu.make_async_copy(
                                src.at[rows(g * G + r), pl.ds(pl.multiple_of(SK - W + col, 128), n * 128)],
                                dst.at[slot, rows(r), pl.ds(pl.multiple_of(col, 128), n * 128)],
                                sem.at[slot]).start(priority=thread)
                            col = col + n * 128

            x_copy = pltpu.make_async_copy(x_hbm, x_v, sem_x)
            x_copy.start()
            issue((wq_hbm, wq_v, sem_wq, q_jobs))
            x_copy.wait()
            x32 = x_v[...].astype(F32)
            lnx = jnp.broadcast_to(_layernorm(x32), (8, D))

            for j in range(HG):
                loop(j * RPH, j * RPH + kv_split, lambda t: kv_round(0, t))
                if j == 0:
                    wait_all(wq_v, sem_wq)
                nc = NG * DH // 128
                t = wq_v[...].reshape(D // 8, HG * nc, 8, 128)
                qc = jnp.concatenate([jnp.dot(lnx, t[:, c].reshape(D, 128), preferred_element_type=F32)
                                      for c in range(j * nc, (j + 1) * nc)], axis=1)
                for i in range(NG):
                    q_v[j * NG + i] = qc[:, i * DH:(i + 1) * DH]
                loop(j * RPH + kv_split, (j + 1) * RPH, lambda t: kv_round(0, t))

            def head(h):
                g, j = h >> (HG.bit_length() - 1), h & (HG - 1)
                slot = g & 1
                more = g + 1 < NG

                def prefetch(lo, hi, part):
                    @pl.when(more)
                    def _():
                        loop(j * RPH + lo, j * RPH + hi, lambda t: kv_round(g + 1, t))

                    for i in range(HG):
                        @pl.when(h == H - HG + i)
                        def _():
                            end = o_first + (2 * i + part) * o_next
                            for job in o_jobs[end - o_next if 2 * i + part else 0:end]:
                                tile_copy(wo_hbm, wo_v, sem_wo, *job)

                prefetch(0, kv_split, 0)

                @pl.when(j == 0)
                def _():
                    wait_all(vbuf.at[slot], sem_v.at[slot])
                    wait_all(kbuf.at[slot], sem_k.at[slot])

                hrows = pl.ds(pl.multiple_of(j * DH, DH), DH)
                qh = q_v[h].astype(BF)
                s = jnp.dot(qh, kbuf[slot, hrows, :], preferred_element_type=F32)
                s = _r(_r(s) * SCALE)
                m = jnp.max(s, axis=-1, keepdims=True)
                e = _r(jnp.exp(_r(s - m)))
                l = _r(jnp.sum(e, axis=-1, keepdims=True))
                p = (e / l).astype(BF)
                prefetch(kv_split, RPH, 1)
                q_v[h] = lax.dot_general(p, vbuf[slot, hrows, :], (((1,), (1,)), ((), ())),
                                         preferred_element_type=F32)

            loop(0, H, head)
            issue((wo_hbm, wo_v, sem_wo, o_jobs[o_first + (2 * HG - 1) * o_next:]))

            def issue_f(lo, hi):
                n = len(w1_jobs)
                issue((w1_hbm, w1_v, sem_w1, w1_jobs[min(lo, n):min(hi, n)]),
                      (w3_hbm, w3_v, sem_w3, w3_jobs[max(lo - n, 0):max(hi - n, 0)]))

            issue_f(0, f_first)
            wait_all(wo_v, sem_wo)
            hs = H // o_steps
            nf = -(-(len(w1_jobs) + len(w3_jobs) - f_first) // o_steps)
            attn = jnp.zeros((8, D), F32)
            for c in range(o_steps):
                o = jnp.concatenate([q_v[c * hs + i] for i in range(hs)], axis=1).astype(BF)
                nt = hs * DH // 8 * DT
                attn = attn + _tile_dot(o, wo_v[c * nt:(c + 1) * nt], DT)
                issue_f(f_first + c * nf, f_first + (c + 1) * nf)
            hres = _r(x32 + _r(attn))
            lnh = _layernorm(hres)

            wait_all(w1_v, sem_w1)
            gate = _r(_tile_dot(lnh, w1_v[...], FT))
            gate = _r(gate * _r(jax.nn.sigmoid(gate)))
            issue(*[(w2_hbm, w2_v, sem_w2.at[i], jobs) for i, jobs in enumerate(w2_jobs)])
            wait_all(w3_v, sem_w3)
            up = _r(_tile_dot(lnh, w3_v[...], FT))
            hm = (gate * up).astype(BF)
            h32 = hm[0:1].astype(F32)
            hcol = {}
            for group in w2_groups[len(w2_mxu):]:
                for r0, n in group:
                    for b in range(r0 // 16, (r0 + n - 1) // 16 + 1):
                        if b not in hcol:
                            hcol[b] = jnp.broadcast_to(h32[:, b * 128:(b + 1) * 128], (128, 128)).T
            out = jnp.zeros((8, D), F32)
            acc = [None] * DT
            for i, group in enumerate(w2_groups):
                for r0, n in group:
                    wait_all(w2_v.at[pl.ds(r0 * DT, n * DT)], sem_w2.at[i])
                for r0, n in group:
                    if i < len(w2_mxu):
                        out = out + _tile_dot(hm[:, r0 * 8:(r0 + n) * 8], w2_v[r0 * DT:(r0 + n) * DT], DT)
                    else:
                        for r in range(r0, r0 + n):
                            hb = hcol[r // 16][r % 16 * 8:(r % 16 + 1) * 8]
                            for c in range(DT):
                                term = hb * w2_v[r * DT + c].astype(F32)
                                acc[c] = term if acc[c] is None else acc[c] + term
            out = out[0:1] + jnp.concatenate([jnp.sum(a, axis=0, keepdims=True) for a in acc], axis=1)
            o_v[...] = (hres[0:1] + _r(out)).astype(o_v.dtype)
            pltpu.make_async_copy(o_v, o_hbm, sem_o).start()

        dma = pltpu.SemaphoreType.DMA
        pl.run_scoped(body, dma(()), dma(()), dma(()), dma((2,)), dma((2,)), dma(()), dma(()),
                      dma((len(w2_groups),)))
        pltpu.make_async_copy(o_v, o_hbm, sem_o).wait()

    @jax.jit
    def run(A_x, A_k_cache, A_v_cache, A_wq, A_wo, B_x, B_w1, B_w3, B_w2):
        del B_x
        x = A_x.reshape(1, D)
        kt = jnp.swapaxes(A_k_cache.reshape(H, SK, DH), 1, 2).reshape(H * DH, SK)
        vt = jnp.swapaxes(A_v_cache.reshape(H, SK, DH), 1, 2).reshape(H * DH, SK)
        tile_buf = lambda a: pltpu.VMEM((a.size // 1024, 8, 128), BF)
        out = pl.pallas_call(
            kernel,
            out_shape=jax.ShapeDtypeStruct((1, D), A_x.dtype),
            in_specs=[pl.BlockSpec(memory_space=pl.ANY)] * 8,
            out_specs=pl.BlockSpec(memory_space=pl.ANY),
            scratch_shapes=[
                pltpu.VMEM((1, D), BF),
                tile_buf(A_wq),
                pltpu.VMEM((H, 8, DH), F32),
                pltpu.VMEM((2, HG * DH, W), BF),
                pltpu.VMEM((2, HG * DH, W), BF),
                tile_buf(A_wo), tile_buf(B_w1), tile_buf(B_w3), tile_buf(B_w2),
                pltpu.VMEM((1, D), BF),
                pltpu.SemaphoreType.DMA(()),
            ],
            compiler_params=pltpu.CompilerParams(vmem_limit_bytes=100 * 1024 * 1024, disable_bounds_checks=True),
        )(x, kt, vt, _tiles(A_wq), _tiles(A_wo), _tiles(B_w1), _tiles(B_w3), _tiles(B_w2))
        return out.reshape(1, 1, D)

    return run


pallas_sequential_preLN__sliding_block_cached__glu_gated_swiglu__decode_kernel = make_kernel()
```

```python
import jax
import jax.numpy as jnp
import numpy as np
from jax import lax
import jax.experimental.pallas as pl
import jax.experimental.pallas.tpu as pltpu

H, DH, SK, D, F = 32, 192, 32768, 640, 1536
W = min(4096, max(256, SK // 4))
BF = jnp.bfloat16
F32 = jnp.float32

CH = 16
CW = CH * 128
HG = 4
NG = H // HG
G = HG * DH // 8
KS = G // 3
ROUNDS = (W // CW) * KS
DT, FT = D // 128, F // 128


def _bf16_round(v):
    u = int(np.float32(v).view(np.uint32))
    u = (u + 0x7FFF + ((u >> 16) & 1)) & 0xFFFF0000
    return float(np.uint32(u).view(np.float32))


SCALE = _bf16_round(DH ** -0.5)
EPS = _bf16_round(1e-5)


def _r(x):
    return x.astype(BF).astype(F32)


def _layernorm(x32):
    m = jnp.mean(x32, axis=-1, keepdims=True)
    c = x32 - m
    v = jnp.mean(c * c, axis=-1, keepdims=True)
    num = _r(x32 - _r(m))
    den = _r(jnp.sqrt(_r(_r(v) + EPS)))
    return (num / den).astype(BF)


def _tiles(a):
    r, c = a.shape
    return a.reshape(r // 8, 8, c // 128, 128).transpose(0, 2, 1, 3).reshape(r // 8 * (c // 128), 8, 128)


def _tile_dot(lhs, tiles, ncol):
    nrb = tiles.shape[0] // ncol
    t = tiles.reshape(nrb, ncol, 8, 128)
    return jnp.concatenate(
        [jnp.dot(lhs, t[:, j].reshape(nrb * 8, 128), preferred_element_type=F32) for j in range(ncol)], axis=1)


def _order(n, streams):
    step = -(-n // streams)
    return [b + step * i for b in range(step) for i in range(streams) if b + step * i < n]


def _cut(t0, n, parts, phase):
    out, end = [], t0 + n
    while t0 < end:
        m = min(end - t0, CH - (t0 - phase) % CH)
        for p in (parts if m == CH else (m,)):
            out.append((t0, p))
            t0 += p
    return out


def _merge(a, b):
    out, ia, ib = [], 0, 0
    while ia < len(a) or ib < len(b):
        if ib >= len(b) or (ia < len(a) and ia * len(b) <= ib * len(a)):
            out += a[ia]
            ia += 1
        else:
            out += b[ib]
            ib += 1
    return out


def _weight_jobs(chunks, streams, off, parts, phase):
    half = chunks // 2

    def second(c):
        if c < chunks - 1 or not phase:
            return _cut(phase + c * CH, CH, parts, phase)
        return [(phase + c * CH, CH - phase), (0, phase)]

    order = _order(half, streams)
    return _merge([[(phase + c * CH, CH, 0)] for c in order],
                  [[(t, n, 1) for t, n in second(half + (c + off) % half)] for c in order])


def make_kernel(q_pat=(5, 2, (6, 10), 0), o_pat=(5, 13, (8, 8), 0), w1_pat=(2, 5, (3, 13), 0),
                w3_pat=(2, 5, (3, 13), 0), w2_pat=((10, 6), 0), kv_pat=(75, 0, (9, 7), 1),
                w2_mxu=(32, 32, 8), w2_vpu=(9, 6, 3, 3, 3),
                kv_split=12, o_first=75, o_next=33, f_first=80, o_steps=4):
    RPH = ROUNDS // HG
    q_jobs = _weight_jobs(D * H * DH // 1024 // CH, *q_pat)
    o_jobs = _weight_jobs(D * H * DH // 1024 // CH, *o_pat)
    w1_jobs = _weight_jobs(D * F // 1024 // CH, *w1_pat)
    w3_jobs = _weight_jobs(D * F // 1024 // CH, *w3_pat)
    assert sum(w2_mxu + w2_vpu) == F // 8 // 2 and all(n % 3 == 0 for n in w2_vpu)
    w2_groups, w2_jobs, rb = [], [], 0
    for i, n in enumerate(w2_mxu + w2_vpu):
        r1 = F // 8 // 2 + rb
        w2_groups.append(((rb, n), (r1, n)))
        if i < len(w2_mxu):
            first = _cut(rb * DT, n * DT, (CH,), w2_pat[1])
            second = _cut(r1 * DT, n * DT, w2_pat[0], w2_pat[1])
        else:
            first = [(r * DT, 3 * DT) for r in range(rb, rb + n, 3)]
            second = [p for r in range(r1, r1 + n) for p in ((r * DT, 2), (r * DT + 2, DT - 2))]
        w2_jobs.append(_merge([[(t, m, 0, t + rb * DT)] for t, m in first],
                              [[(t, m, 1, t + (2 * rb + n - r1) * DT)] for t, m in second]))
        rb += n

    def kernel(x_hbm, kt_hbm, vt_hbm, wq_hbm, wo_hbm, w1_hbm, w3_hbm, w2_hbm, o_hbm,
               x_v, wq_v, q_v, kbuf, vbuf, wo_v, w1_v, w3_v, w2_v, o_v, sem_o):

        def body(sem_x, sem_wq, sem_wo, sem_k, sem_v, sem_w1, sem_w3, sem_w2):
            def wait_all(ref, sem):
                pltpu.make_async_copy(ref, ref, sem).wait()

            def loop(lo, hi, fn):
                lax.fori_loop(lo, hi, lambda i, c: (fn(i), c)[1], 0)

            def wrap(i, n):
                return jnp.where(i >= n, i - n, i)

            def rows(rb):
                return pl.ds(pl.multiple_of(rb * 8, 8), 8)

            def tile_copy(src, dst, sem, t0, n, thread, d0=None):
                pltpu.make_async_copy(src.at[pl.ds(t0, n)], dst.at[pl.ds(t0 if d0 is None else d0, n)],
                                      sem).start(priority=thread)

            def issue(*runs):
                runs = [run for run in runs if run[3]]

                def step(i):
                    for n, (src, dst, sem, jobs) in enumerate(runs):
                        @pl.when(i == n)
                        def _():
                            for job in jobs:
                                tile_copy(src, dst, sem, *job)

                if runs:
                    loop(0, max(len(runs), 2), step)

            def kv_round(g, t):
                off, flip, parts, swap = kv_pat
                slot, half, b = g & 1, t >> (KS.bit_length() - 1), t & (KS - 1)
                for i in range(3):
                    k = 2 * (3 * b + i)
                    rb = jnp.where(k >= G, k - (G - 1), k)
                    for thread, r, c, pieces in ((0, rb, half, (CH,)), (1, wrap(rb + off, G), half ^ flip, parts)):
                        src, dst, sem = ((kt_hbm, kbuf, sem_k), (vt_hbm, vbuf, sem_v))[thread ^ swap]
                        col = c * CW
                        for n in pieces:
                            pltpu.make_async_copy(
                                src.at[rows(g * G + r), pl.ds(pl.multiple_of(SK - W + col, 128), n * 128)],
                                dst.at[slot, rows(r), pl.ds(pl.multiple_of(col, 128), n * 128)],
                                sem.at[slot]).start(priority=thread)
                            col = col + n * 128

            x_copy = pltpu.make_async_copy(x_hbm, x_v, sem_x)
            x_copy.start()
            issue((wq_hbm, wq_v, sem_wq, q_jobs))
            x_copy.wait()
            x32 = x_v[...].astype(F32)
            lnx = jnp.broadcast_to(_layernorm(x32), (8, D))

            for j in range(HG):
                loop(j * RPH, j * RPH + kv_split, lambda t: kv_round(0, t))
                if j == 0:
                    wait_all(wq_v, sem_wq)
                nc = NG * DH // 128
                t = wq_v[...].reshape(D // 8, HG * nc, 8, 128)
                qc = jnp.concatenate([jnp.dot(lnx, t[:, c].reshape(D, 128), preferred_element_type=F32)
                                      for c in range(j * nc, (j + 1) * nc)], axis=1)
                for i in range(NG):
                    q_v[j * NG + i] = qc[:, i * DH:(i + 1) * DH]
                loop(j * RPH + kv_split, (j + 1) * RPH, lambda t: kv_round(0, t))

            def head(h):
                g, j = h >> (HG.bit_length() - 1), h & (HG - 1)
                slot = g & 1
                more = g + 1 < NG

                def prefetch(lo, hi, part):
                    @pl.when(more)
                    def _():
                        loop(j * RPH + lo, j * RPH + hi, lambda t: kv_round(g + 1, t))

                    for i in range(HG):
                        @pl.when(h == H - HG + i)
                        def _():
                            end = o_first + (2 * i + part) * o_next
                            for job in o_jobs[end - o_next if 2 * i + part else 0:end]:
                                tile_copy(wo_hbm, wo_v, sem_wo, *job)

                prefetch(0, kv_split, 0)

                @pl.when(j == 0)
                def _():
                    wait_all(vbuf.at[slot], sem_v.at[slot])
                    wait_all(kbuf.at[slot], sem_k.at[slot])

                hrows = pl.ds(pl.multiple_of(j * DH, DH), DH)
                qh = q_v[h].astype(BF)
                s = jnp.dot(qh, kbuf[slot, hrows, :], preferred_element_type=F32)
                s = _r(_r(s) * SCALE)
                m = jnp.max(s, axis=-1, keepdims=True)
                e = _r(jnp.exp(_r(s - m)))
                l = _r(jnp.sum(e, axis=-1, keepdims=True))
                p = (e / l).astype(BF)
                prefetch(kv_split, RPH, 1)
                q_v[h] = lax.dot_general(p, vbuf[slot, hrows, :], (((1,), (1,)), ((), ())),
                                         preferred_element_type=F32)

            loop(0, H, head)
            issue((wo_hbm, wo_v, sem_wo, o_jobs[o_first + (2 * HG - 1) * o_next:]))

            def issue_f(lo, hi):
                n = len(w1_jobs)
                issue((w1_hbm, w1_v, sem_w1, w1_jobs[min(lo, n):min(hi, n)]),
                      (w3_hbm, w3_v, sem_w3, w3_jobs[max(lo - n, 0):max(hi - n, 0)]))

            issue_f(0, f_first)
            wait_all(wo_v, sem_wo)
            hs = H // o_steps
            nf = -(-(len(w1_jobs) + len(w3_jobs) - f_first) // o_steps)
            attn = jnp.zeros((8, D), F32)
            for c in range(o_steps):
                o = jnp.concatenate([q_v[c * hs + i] for i in range(hs)], axis=1).astype(BF)
                nt = hs * DH // 8 * DT
                attn = attn + _tile_dot(o, wo_v[c * nt:(c + 1) * nt], DT)
                issue_f(f_first + c * nf, f_first + (c + 1) * nf)
            hres = _r(x32 + _r(attn))
            lnh = _layernorm(hres)

            wait_all(w1_v, sem_w1)
            gate = _r(_tile_dot(lnh, w1_v[...], FT))
            gate = _r(gate * _r(jax.nn.sigmoid(gate)))
            issue(*[(w2_hbm, w2_v, sem_w2.at[i], jobs) for i, jobs in enumerate(w2_jobs)])
            wait_all(w3_v, sem_w3)
            up = _r(_tile_dot(lnh, w3_v[...], FT))
            hm = (gate * up).astype(BF)
            h32 = hm[0:1].astype(F32)
            hcol = {}
            for group in w2_groups[len(w2_mxu):]:
                for r0, n in group:
                    for b in range(r0 // 16, (r0 + n - 1) // 16 + 1):
                        if b not in hcol:
                            hcol[b] = jnp.broadcast_to(h32[:, b * 128:(b + 1) * 128], (128, 128)).T
            out = jnp.zeros((8, D), F32)
            acc = [None] * DT
            for i, group in enumerate(w2_groups):
                rb, n = group[0]
                wait_all(w2_v.at[pl.ds(2 * rb * DT, 2 * n * DT)], sem_w2.at[i])
                for (r0, _), v0 in zip(group, (2 * rb, 2 * rb + n)):
                    if i < len(w2_mxu):
                        out = out + _tile_dot(hm[:, r0 * 8:(r0 + n) * 8], w2_v[v0 * DT:(v0 + n) * DT], DT)
                    else:
                        for r in range(r0, r0 + n):
                            hb = hcol[r // 16][r % 16 * 8:(r % 16 + 1) * 8]
                            for c in range(DT):
                                term = hb * w2_v[(v0 + r - r0) * DT + c].astype(F32)
                                acc[c] = term if acc[c] is None else acc[c] + term
            out = out[0:1] + jnp.concatenate([jnp.sum(a, axis=0, keepdims=True) for a in acc], axis=1)
            o_v[...] = (hres[0:1] + _r(out)).astype(o_v.dtype)
            pltpu.make_async_copy(o_v, o_hbm, sem_o).start()

        dma = pltpu.SemaphoreType.DMA
        pl.run_scoped(body, dma(()), dma(()), dma(()), dma((2,)), dma((2,)), dma(()), dma(()),
                      dma((len(w2_groups),)))
        pltpu.make_async_copy(o_v, o_hbm, sem_o).wait()

    @jax.jit
    def run(A_x, A_k_cache, A_v_cache, A_wq, A_wo, B_x, B_w1, B_w3, B_w2):
        del B_x
        x = A_x.reshape(1, D)
        kt = jnp.swapaxes(A_k_cache.reshape(H, SK, DH), 1, 2).reshape(H * DH, SK)
        vt = jnp.swapaxes(A_v_cache.reshape(H, SK, DH), 1, 2).reshape(H * DH, SK)
        tile_buf = lambda a: pltpu.VMEM((a.size // 1024, 8, 128), BF)
        out = pl.pallas_call(
            kernel,
            out_shape=jax.ShapeDtypeStruct((1, D), A_x.dtype),
            in_specs=[pl.BlockSpec(memory_space=pl.ANY)] * 8,
            out_specs=pl.BlockSpec(memory_space=pl.ANY),
            scratch_shapes=[
                pltpu.VMEM((1, D), BF),
                tile_buf(A_wq),
                pltpu.VMEM((H, 8, DH), F32),
                pltpu.VMEM((2, HG * DH, W), BF),
                pltpu.VMEM((2, HG * DH, W), BF),
                tile_buf(A_wo), tile_buf(B_w1), tile_buf(B_w3), tile_buf(B_w2),
                pltpu.VMEM((1, D), BF),
                pltpu.SemaphoreType.DMA(()),
            ],
            compiler_params=pltpu.CompilerParams(vmem_limit_bytes=100 * 1024 * 1024, disable_bounds_checks=True),
        )(x, kt, vt, _tiles(A_wq), _tiles(A_wo), _tiles(B_w1), _tiles(B_w3), _tiles(B_w2))
        return out.reshape(1, 1, D)

    return run


pallas_sequential_preLN__sliding_block_cached__glu_gated_swiglu__decode_kernel = make_kernel()
```
